```python
import os as _os
_os.environ.setdefault("JAX_PLATFORMS", "cpu")
import jax
import jax.numpy as jnp

def _softmax(x, axis=-1):
    return jax.nn.softmax(x, axis=axis)
def _gelu(x):
    return jax.nn.gelu(x, approximate=True)
def _silu(x):
    return jax.nn.silu(x)
def _sigmoid(x):
    return jax.nn.sigmoid(x)
def _layernorm(x, axis=-1, eps=1e-5):
    m = jnp.mean(x, axis=axis, keepdims=True)
    v = jnp.var(x, axis=axis, keepdims=True)
    return (x - m) / jnp.sqrt(v + eps)
def _scatter_add(tgt, idx, src, axis=0):
    return tgt.at[idx].add(src)
def _segment_sum(src, seg, n):
    return jax.ops.segment_sum(src, seg, n)
class _Rng:
    def __init__(self, key):
        self._k = key
    def _next(self):
        self._k, sub = jax.random.split(self._k)
        return sub
    def normal(self, shape):
        return jax.random.normal(self._next(), shape, dtype=jnp.bfloat16)
    def randint(self, lo, hi, shape):
        return jax.random.randint(self._next(), shape, lo, hi, dtype=jnp.int32)
    def uniform(self, shape, lo=0.0, hi=1.0):
        return jax.random.uniform(self._next(), shape, jnp.bfloat16, lo, hi)
    def permutation(self, n):
        return jax.random.permutation(self._next(), n)


kernel_name = 'interleave_layers__linear_kernel_hedgehog__dense_activation_silu__prompt'

def setup_inputs():
    _rng = _Rng(jax.random.key(int.from_bytes(__import__("os").urandom(4), "little")))
    _w = (lambda a: (lambda t: t.astype(jnp.bfloat16) if jnp.issubdtype(t.dtype, jnp.floating) else t)(jnp.asarray(a)))
    def _A_setup():
        B, S, D, H = 1, 2048, 640, 32
        Dh = D // H
        return {
            "x": _w((lambda *s: _rng.normal(s) * 0.05)(B, S, D)),
            "wqkv": _w((lambda *s: _rng.normal(s) * 0.4)(D, 3 * D)),
            "w_phi": _w((lambda *s: _rng.normal(s) * 0.4)(H, Dh, Dh) * (Dh ** -0.5)),
            "wo": _w((lambda *s: _rng.normal(s) * 0.05)(D, D)),
        }
    _A_in = _A_setup()

    def _B_setup():
        B, S, D, F = 1, 2048, 640, 1728
        return {
            "x": _w((lambda *s: _rng.normal(s) * 0.05)(B, S, D)),
            "w1": _w((lambda *s: _rng.normal(s) * 1.6)(D, F) * (D ** -0.5)),
            "w2": _w((lambda *s: _rng.normal(s) * 1.6)(F, D) * (F ** -0.5)),
        }
    _B_in = _B_setup()

    return {
        "A_x": _A_in["x"],
        "A_wqkv": _A_in["wqkv"],
        "A_w_phi": _A_in["w_phi"],
        "A_wo": _A_in["wo"],
        "B_x": _B_in["x"],
        "B_w1": _B_in["w1"],
        "B_w2": _B_in["w2"],
    }

def reference(A_x, A_wqkv, A_w_phi, A_wo, B_x, B_w1, B_w2):
    def _A_ref(x, wqkv, w_phi, wo):
        B, S, D = x.shape
        H = 32; Dh = D // H
        qkv = (lambda x, *d: x.transpose(*d))((x @ wqkv).reshape(B, S, 3, H, Dh), 2, 0, 3, 1, 4)
        q, k, v = qkv[0], qkv[1], qkv[2]
        pq = jnp.einsum("bhsd,hdf->bhsf", q, w_phi)
        pk = jnp.einsum("bhsd,hdf->bhsf", k, w_phi)
        phi_q = jnp.concatenate([_softmax(pq, axis=-1), _softmax(-pq, axis=-1)], axis=-1)
        phi_k = jnp.concatenate([_softmax(pk, axis=-1), _softmax(-pk, axis=-1)], axis=-1)
        kv = jnp.einsum("bhsf,bhsd->bhfd", phi_k, v)
        z  = jnp.einsum("bhsf->bhf", phi_k)
        num = jnp.einsum("bhqf,bhfd->bhqd", phi_q, kv)
        den = jnp.einsum("bhqf,bhf->bhq", phi_q, z)[..., None] + 1e-6
        o = num / den
        return (lambda x, *d: x.transpose(*d))(o, 0, 2, 1, 3).reshape(B, S, D) @ wo

    def _B_ref(x, w1, w2):
        h = jnp.einsum("bsd,df->bsf", x, w1)
        h = _silu(h)
        out = jnp.einsum("bsf,fd->bsd", h, w2)
        return out

    x = A_x
    x = x + _A_ref(_layernorm(x, axis=-1), A_wqkv, A_w_phi, A_wo)
    x = x + _B_ref(_layernorm(x, axis=-1), B_w1, B_w2)
    x = x + _A_ref(_layernorm(x, axis=-1), A_wqkv, A_w_phi, A_wo)
    x = x + _B_ref(_layernorm(x, axis=-1), B_w1, B_w2)
    return x
```

```python
import functools

import jax
import jax.numpy as jnp
from jax import lax
import jax.experimental.pallas as pl
import jax.experimental.pallas.tpu as pltpu

S = 2048
D = 640
H = 32
DH = D // H
F = 1728
HG = 8
NHG = H // HG
GV = HG * DH
GF = 2 * GV

TB = 256
NB = S // TB
NSTEP = 3 * NB
LN_EPS = 1e-5
DEN_EPS = 1e-6

_NT = (((1,), (1,)), ((), ()))


def _nt(a, b):
    return lax.dot_general(a, b, _NT, preferred_element_type=jnp.float32)


def _nn(a, b):
    return jnp.dot(a, b, preferred_element_type=jnp.float32)


def _layernorm_bf16(x):
    m = jnp.mean(x, axis=-1, keepdims=True)
    xc = x - m
    v = jnp.mean(xc * xc, axis=-1, keepdims=True)
    return (xc * lax.rsqrt(v + LN_EPS)).astype(jnp.bfloat16)


def _features_t(p):
    t = p.shape[1]
    p4 = p.reshape(NHG, DH, HG, t)
    mx = jnp.max(p4, axis=1, keepdims=True)
    mn = jnp.min(p4, axis=1, keepdims=True)
    ep = jnp.exp(p4 - mx)
    en = jnp.exp(mn - p4)
    rp = 1.0 / jnp.sum(ep, axis=1, keepdims=True)
    rn = 1.0 / jnp.sum(en, axis=1, keepdims=True)
    phi = jnp.concatenate([ep * rp, en * rn], axis=1)
    return phi.reshape(2 * D, t).astype(jnp.bfloat16)


def _kernel(x_ref, wqkv_hbm, wphi_ref, wo_hbm, w1t_hbm, w2_hbm, o_ref,
            wqkv_ref, wo_ref, w1t_ref, w2_ref, sems,
            wt_ref, wflat_ref, phiq_ref, xs_ref, qkvt_ref,
            kvt_acc_ref, z_acc_ref, kvt_ref, zb_ref):
    t_id = pl.program_id(0)

    def wcopy(k):
        src, dst = ((wqkv_hbm, wqkv_ref), (wo_hbm, wo_ref),
                    (w1t_hbm, w1t_ref), (w2_hbm, w2_ref))[k]
        return pltpu.make_async_copy(src, dst, sems.at[k])

    def prep():
        wflat_ref[...] = jnp.zeros_like(wflat_ref)
        for h in range(H):
            wflat_ref[pl.ds(h * DH, DH), pl.ds(0, DH)] = (
                wphi_ref[h].astype(jnp.float32))
        wflat = wflat_ref[...].astype(jnp.bfloat16)
        crow = lax.broadcasted_iota(jnp.int32, (D, 128), 0)
        dcol = lax.broadcasted_iota(jnp.int32, (D, 128), 1)
        sel = jnp.where((crow % GV) // HG == dcol, 1.0, 0.0).astype(jnp.bfloat16)
        pt = _nt(sel, wflat)
        crow = lax.broadcasted_iota(jnp.int32, (D, D), 0)
        rcol = lax.broadcasted_iota(jnp.int32, (D, D), 1)
        head_c = (crow // GV) * HG + crow % HG
        head_r = rcol // DH
        pt = jnp.where(head_c == head_r, pt, 0.0).astype(jnp.bfloat16)
        wcopy(0).wait()
        wt_ref[pl.ds(2 * D, D), :] = wqkv_ref[:, pl.ds(2 * D, D)].T
        for part in range(2):
            for g in range(NHG):
                wt_ref[pl.ds(part * D + g * GV, GV), :] = _nt(
                    pt[g * GV:(g + 1) * GV, g * 128:g * 128 + 256],
                    wqkv_ref[:, pl.ds(part * D + g * 128, 256)],
                ).astype(jnp.bfloat16)

    def reset_acc():
        kvt_acc_ref[...] = jnp.zeros_like(kvt_acc_ref)
        z_acc_ref[...] = jnp.zeros_like(z_acc_ref)

    def finalize():
        crow = lax.broadcasted_iota(jnp.int32, (GV, GF), 0)
        fcol = lax.broadcasted_iota(jnp.int32, (GV, GF), 1)
        same_head = (crow // DH) == (fcol % HG)
        for g in range(NHG):
            kvt_ref[g] = jnp.where(same_head, kvt_acc_ref[g], 0.0).astype(
                jnp.bfloat16)
        z = jnp.sum(z_acc_ref[...], axis=1, keepdims=True)
        zb_ref[...] = jnp.broadcast_to(z, zb_ref.shape)

    def stage_a(blk):
        x0 = xs_ref[blk]
        phiq = phiq_ref[blk].astype(jnp.float32)
        zb = zb_ref[...]
        zb_t = jnp.concatenate([zb] * (TB // 128), axis=1)
        pz = (phiq * zb_t).reshape(NHG, 2 * DH, HG, TB)
        den = jnp.sum(pz, axis=1, keepdims=True) + DEN_EPS
        phin = (phiq.reshape(NHG, 2 * DH, HG, TB) / den).reshape(2 * D, TB)
        phin = phin.astype(jnp.bfloat16)
        ot = jnp.concatenate(
            [_nn(kvt_ref[g], phin[g * GF:(g + 1) * GF, :]) for g in range(NHG)],
            axis=0)
        o = ot.astype(jnp.bfloat16).T
        x1 = x0 + _nn(o, wo_ref[...])
        xn1 = _layernorm_bf16(x1)
        hpre = _nt(xn1, w1t_ref[...])
        hact = (hpre * jax.nn.sigmoid(hpre)).astype(jnp.bfloat16)
        x2 = x1 + _nn(hact, w2_ref[...])
        xs_ref[blk] = x2

    def stage_bmm(blk):
        xn = _layernorm_bf16(xs_ref[blk])
        qkvt_ref[...] = _nt(wt_ref[...], xn)

    def stage_bfeat(blk):
        phiq_ref[blk] = _features_t(qkvt_ref[pl.ds(0, D), :])
        phik = _features_t(qkvt_ref[pl.ds(D, D), :])
        vt = qkvt_ref[pl.ds(2 * D, D), :].astype(jnp.bfloat16)
        for g in range(NHG):
            kvt_acc_ref[g] += _nt(vt[g * GV:(g + 1) * GV, :],
                                  phik[g * GF:(g + 1) * GF, :])
        phik32 = phik.astype(jnp.float32)
        zpart = phik32[:, 0:128]
        for j in range(1, TB // 128):
            zpart = zpart + phik32[:, j * 128:(j + 1) * 128]
        z_acc_ref[...] += zpart

    blk = t_id % NB

    @pl.when(t_id == 0)
    def _():
        for k in range(4):
            wcopy(k).start()
        prep()
        reset_acc()

    @pl.when(t_id < NB)
    def _():
        xs_ref[blk] = x_ref[...].astype(jnp.float32)

    @pl.when(jnp.logical_or(t_id == NB, t_id == 2 * NB))
    def _():
        stage_bfeat(NB - 1)
        finalize()
        reset_acc()

    @pl.when(t_id == NB)
    def _():
        for k in range(1, 4):
            wcopy(k).wait()

    @pl.when(t_id >= NB)
    def _():
        stage_a(blk)

    @pl.when(t_id >= 2 * NB)
    def _():
        o_ref[...] = xs_ref[blk].astype(o_ref.dtype)

    @pl.when(jnp.logical_and(blk == 0, t_id < 2 * NB))
    def _():
        stage_bmm(blk)

    @pl.when(jnp.logical_and(blk > 0, t_id < 2 * NB))
    def _():
        stage_bfeat(blk - 1)
        stage_bmm(blk)


@jax.jit
def pallas_interleave_layers__linear_kernel_hedgehog__dense_activation_silu__prompt_kernel(
    A_x: jax.Array,
    A_wqkv: jax.Array,
    A_w_phi: jax.Array,
    A_wo: jax.Array,
    B_x: jax.Array,
    B_w1: jax.Array,
    B_w2: jax.Array,
):
    del B_x
    x2d = A_x.reshape(S, D)
    w1t = B_w1.T

    hbm = pl.BlockSpec(memory_space=pl.ANY)
    grid_spec = pltpu.PrefetchScalarGridSpec(
        num_scalar_prefetch=0,
        grid=(NSTEP,),
        in_specs=[
            pl.BlockSpec((TB, D), lambda t: (jnp.minimum(t, NB - 1), 0)),
            hbm,
            pl.BlockSpec((H, DH, DH), lambda t: (0, 0, 0)),
            hbm, hbm, hbm,
        ],
        out_specs=pl.BlockSpec((TB, D), lambda t: (jnp.maximum(t - 2 * NB, 0), 0)),
        scratch_shapes=[
            pltpu.VMEM((D, 3 * D), jnp.bfloat16),
            pltpu.VMEM((D, D), jnp.bfloat16),
            pltpu.VMEM((F, D), jnp.bfloat16),
            pltpu.VMEM((F, D), jnp.bfloat16),
            pltpu.SemaphoreType.DMA((4,)),
            pltpu.VMEM((3 * D, D), jnp.bfloat16),
            pltpu.VMEM((D, 128), jnp.float32),
            pltpu.VMEM((NB, 2 * D, TB), jnp.bfloat16),
            pltpu.VMEM((NB, TB, D), jnp.float32),
            pltpu.VMEM((3 * D, TB), jnp.float32),
            pltpu.VMEM((NHG, GV, GF), jnp.float32),
            pltpu.VMEM((2 * D, 128), jnp.float32),
            pltpu.VMEM((NHG, GV, GF), jnp.bfloat16),
            pltpu.VMEM((2 * D, 128), jnp.float32),
        ],
    )
    out = pl.pallas_call(
        _kernel,
        grid_spec=grid_spec,
        out_shape=jax.ShapeDtypeStruct((S, D), jnp.bfloat16),
        compiler_params=pltpu.CompilerParams(
            dimension_semantics=("arbitrary",),
            vmem_limit_bytes=100 * 1024 * 1024,
        ),
    )(x2d, A_wqkv, A_w_phi, A_wo, w1t, B_w2)
    return out.reshape(1, S, D)
```

```python
import functools

import jax
import jax.numpy as jnp
from jax import lax
import jax.experimental.pallas as pl
import jax.experimental.pallas.tpu as pltpu

S = 2048
D = 640
H = 32
DH = D // H
F = 1728
G4 = 4
NG = H // G4
GV = G4 * DH
GF = 2 * GV
NT10 = GV // 8

TB = 512
NB = S // TB
NL = TB // 128
NSTEP = 3 * NB
LOG2E = 1.4426950408889634
LN_EPS = 1e-5
DEN_EPS = 1e-6

_NT = (((1,), (1,)), ((), ()))


def _nt(a, b):
    return lax.dot_general(a, b, _NT, preferred_element_type=jnp.float32)


def _nn(a, b):
    return jnp.dot(a, b, preferred_element_type=jnp.float32)


def _layernorm_bf16(x):
    m = jnp.mean(x, axis=-1, keepdims=True)
    xc = x - m
    v = jnp.mean(xc * xc, axis=-1, keepdims=True)
    return (xc * lax.rsqrt(v + LN_EPS)).astype(jnp.bfloat16)


def _fold_halves(x, op):
    return op(x, pltpu.roll(x, 4, 0))


def _feature_unit(p):
    p3 = p.reshape(NT10, 8, 128)
    mx = _fold_halves(jnp.max(p3, axis=0), jnp.maximum)
    mn = _fold_halves(jnp.min(p3, axis=0), jnp.minimum)
    ep = jnp.exp2(p3 - mx[None])
    en = jnp.exp2(mn[None] - p3)
    rp = 1.0 / _fold_halves(jnp.sum(ep, axis=0), jnp.add)
    rn = 1.0 / _fold_halves(jnp.sum(en, axis=0), jnp.add)
    phi = jnp.concatenate([ep * rp[None], en * rn[None]], axis=0)
    return phi.reshape(GF, 128)


def _kernel(x_ref, wqkv_hbm, wphi_ref, wo_hbm, w1t_hbm, w2_hbm, o_ref,
            wqkv_ref, wo_ref, w1t_ref, w2_ref, sems,
            wt_ref, wflat_ref, phiq_ref, xs_ref, qkvt_ref, phik_ref, vt_ref, phin_ref,
            kvt_acc_ref, z_acc_ref, kvt_ref, zb_ref):
    t_id = pl.program_id(0)

    def wcopy(k):
        if k < 3:
            src = wqkv_hbm.at[:, pl.ds(k * D, D)]
            dst = wqkv_ref.at[:, pl.ds(k * D, D)]
        else:
            src, dst = ((wo_hbm, wo_ref), (w1t_hbm, w1t_ref),
                        (w2_hbm, w2_ref))[k - 3]
        return pltpu.make_async_copy(src, dst, sems.at[k])

    def prep():
        wflat_ref[...] = jnp.zeros_like(wflat_ref)
        for h in range(H):
            wflat_ref[pl.ds(h * DH, DH), pl.ds(0, DH)] = (
                wphi_ref[h].astype(jnp.float32))
        wflat = wflat_ref[...].astype(jnp.bfloat16)
        crow = lax.broadcasted_iota(jnp.int32, (2 * GV, 128), 0)
        dcol = lax.broadcasted_iota(jnp.int32, (2 * GV, 128), 1)
        rem = crow % GV
        dsel = (rem // 8) * 2 + (rem % 8) // 4
        sel = jnp.where(dsel == dcol, 1.0, 0.0).astype(jnp.bfloat16)
        crow = lax.broadcasted_iota(jnp.int32, (2 * GV, 256), 0)
        rcol = lax.broadcasted_iota(jnp.int32, (2 * GV, 256), 1)
        head_c = (crow // GV) * G4 + crow % G4
        pts = []
        for g in range(NG // 2):
            ptw = _nt(sel, wflat[g * 128:g * 128 + 256, :])
            head_r = (rcol + g * 128) // DH - g * 2 * G4
            pts.append(jnp.where(head_c == head_r, ptw * LOG2E, 0.0).astype(
                jnp.bfloat16))
        for part in range(2):
            wcopy(part).wait()
            for g in range(NG // 2):
                wt_ref[pl.ds(part * D + g * 2 * GV, 2 * GV), :] = _nt(
                    pts[g], wqkv_ref[:, pl.ds(part * D + g * 128, 256)],
                ).astype(jnp.bfloat16)
        wcopy(2).wait()
        wt_ref[pl.ds(2 * D, D), :] = wqkv_ref[:, pl.ds(2 * D, D)].T

    def reset_acc():
        kvt_acc_ref[...] = jnp.zeros_like(kvt_acc_ref)
        z_acc_ref[...] = jnp.zeros_like(z_acc_ref)

    def finalize():
        crow = lax.broadcasted_iota(jnp.int32, (GV, GF), 0)
        fcol = lax.broadcasted_iota(jnp.int32, (GV, GF), 1)
        same_head = (crow // DH) == (fcol % G4)
        for g in range(NG):
            kvt_ref[g] = jnp.where(same_head, kvt_acc_ref[g], 0.0).astype(
                jnp.bfloat16)
        z = jnp.sum(z_acc_ref[...], axis=1, keepdims=True)
        zb_ref[...] = jnp.broadcast_to(z, zb_ref.shape)

    def stage_a(blk):
        for g in range(NG):
            zt = zb_ref[pl.ds(g * GF, GF), :].reshape(2 * NT10, 8, 128)
            for j in range(NL):
                pq = phiq_ref[blk, pl.ds(g * GF, GF), pl.ds(j * 128, 128)]
                pq = pq.astype(jnp.float32).reshape(2 * NT10, 8, 128)
                den = _fold_halves(jnp.sum(pq * zt, axis=0), jnp.add) + DEN_EPS
                pn = (pq * (1.0 / den)[None]).reshape(GF, 128)
                phin_ref[pl.ds(g * GF, GF), pl.ds(j * 128, 128)] = (
                    pn.astype(jnp.bfloat16))
        ot = jnp.concatenate(
            [_nn(kvt_ref[g], phin_ref[pl.ds(g * GF, GF), :])
             for g in range(NG)], axis=0)
        o = ot.astype(jnp.bfloat16).T
        x1 = xs_ref[blk] + _nn(o, wo_ref[...])
        xn1 = _layernorm_bf16(x1)
        hpre = _nt(xn1, w1t_ref[...])
        hact = (hpre * jax.nn.sigmoid(hpre)).astype(jnp.bfloat16)
        x2 = x1 + _nn(hact, w2_ref[...])
        xs_ref[blk] = x2

    def stage_bmm(blk):
        xn = _layernorm_bf16(xs_ref[blk])
        qkvt_ref[...] = _nt(wt_ref[...], xn)

    def feat_q(blk):
        for g in range(NG):
            for j in range(NL):
                phi = _feature_unit(
                    qkvt_ref[pl.ds(g * GV, GV), pl.ds(j * 128, 128)])
                phiq_ref[blk, pl.ds(g * GF, GF), pl.ds(j * 128, 128)] = (
                    phi.astype(jnp.bfloat16))

    def feat_kv():
        for g in range(NG):
            zsum = None
            for j in range(NL):
                phi = _feature_unit(
                    qkvt_ref[pl.ds(D + g * GV, GV), pl.ds(j * 128, 128)])
                phik_ref[pl.ds(g * GF, GF), pl.ds(j * 128, 128)] = (
                    phi.astype(jnp.bfloat16))
                zsum = phi if zsum is None else zsum + phi
            z_acc_ref[pl.ds(g * GF, GF), :] += zsum
        vt_ref[...] = qkvt_ref[pl.ds(2 * D, D), :].astype(jnp.bfloat16)

    def stage_bfeat(blk):
        feat_q(blk)
        feat_kv()

    def stage_bkv():
        for g in range(NG):
            kvt_acc_ref[g] += _nt(vt_ref[pl.ds(g * GV, GV), :],
                                  phik_ref[pl.ds(g * GF, GF), :])

    def zero_kv_operands():
        phik_ref[...] = jnp.zeros_like(phik_ref)
        vt_ref[...] = jnp.zeros_like(vt_ref)

    blk = t_id % NB

    @pl.when(t_id == 0)
    def _():
        for k in range(3):
            wcopy(k).start()
        reset_acc()
        zero_kv_operands()
        prep()
        for k in range(3, 6):
            wcopy(k).start()

    @pl.when(t_id < NB)
    def _():
        xs_ref[blk] = x_ref[...].astype(jnp.float32)

    @pl.when(jnp.logical_or(t_id == NB, t_id == 2 * NB))
    def _():
        stage_bkv()
        feat_kv()
        stage_bkv()
        feat_q(NB - 1)
        finalize()
        reset_acc()
        zero_kv_operands()

    @pl.when(t_id == NB)
    def _():
        for k in range(3, 6):
            wcopy(k).wait()

    @pl.when(t_id >= NB)
    def _():
        stage_a(blk)

    @pl.when(t_id >= 2 * NB)
    def _():
        o_ref[...] = xs_ref[blk].astype(o_ref.dtype)

    @pl.when(jnp.logical_and(blk == 0, t_id < 2 * NB))
    def _():
        stage_bmm(blk)

    @pl.when(jnp.logical_and(blk > 0, t_id < 2 * NB))
    def _():
        stage_bkv()
        stage_bfeat(blk - 1)
        stage_bmm(blk)


@jax.jit
def pallas_interleave_layers__linear_kernel_hedgehog__dense_activation_silu__prompt_kernel(
    A_x: jax.Array,
    A_wqkv: jax.Array,
    A_w_phi: jax.Array,
    A_wo: jax.Array,
    B_x: jax.Array,
    B_w1: jax.Array,
    B_w2: jax.Array,
):
    del B_x
    x2d = A_x.reshape(S, D)
    w1t = B_w1.T

    hbm = pl.BlockSpec(memory_space=pl.ANY)
    grid_spec = pltpu.PrefetchScalarGridSpec(
        num_scalar_prefetch=0,
        grid=(NSTEP,),
        in_specs=[
            pl.BlockSpec((TB, D), lambda t: (jnp.minimum(t, NB - 1), 0)),
            hbm,
            pl.BlockSpec((H, DH, DH), lambda t: (0, 0, 0)),
            hbm, hbm, hbm,
        ],
        out_specs=pl.BlockSpec((TB, D), lambda t: (jnp.maximum(t - 2 * NB, 0), 0)),
        scratch_shapes=[
            pltpu.VMEM((D, 3 * D), jnp.bfloat16),
            pltpu.VMEM((D, D), jnp.bfloat16),
            pltpu.VMEM((F, D), jnp.bfloat16),
            pltpu.VMEM((F, D), jnp.bfloat16),
            pltpu.SemaphoreType.DMA((6,)),
            pltpu.VMEM((3 * D, D), jnp.bfloat16),
            pltpu.VMEM((D, 128), jnp.float32),
            pltpu.VMEM((NB, 2 * D, TB), jnp.bfloat16),
            pltpu.VMEM((NB, TB, D), jnp.float32),
            pltpu.VMEM((3 * D, TB), jnp.float32),
            pltpu.VMEM((2 * D, TB), jnp.bfloat16),
            pltpu.VMEM((D, TB), jnp.bfloat16),
            pltpu.VMEM((2 * D, TB), jnp.bfloat16),
            pltpu.VMEM((NG, GV, GF), jnp.float32),
            pltpu.VMEM((2 * D, 128), jnp.float32),
            pltpu.VMEM((NG, GV, GF), jnp.bfloat16),
            pltpu.VMEM((2 * D, 128), jnp.float32),
        ],
    )
    out = pl.pallas_call(
        _kernel,
        grid_spec=grid_spec,
        out_shape=jax.ShapeDtypeStruct((S, D), jnp.bfloat16),
        compiler_params=pltpu.CompilerParams(
            dimension_semantics=("arbitrary",),
            vmem_limit_bytes=100 * 1024 * 1024,
        ),
    )(x2d, A_wqkv, A_w_phi, A_wo, w1t, B_w2)
    return out.reshape(1, S, D)
```

```python
import jax
import jax.numpy as jnp
from jax import lax
import jax.experimental.pallas as pl
import jax.experimental.pallas.tpu as pltpu

S = 2048
D = 640
H = 32
DH = D // H
F = 1728
G4 = 4
NG = H // G4
GV = G4 * DH
GF = 2 * GV
NT10 = GV // 8

TB = 512
NB = S // TB
NL = TB // 128
NSTEP = 3 * NB
LOG2E = 1.4426950408889634
LN_EPS = 1e-5
DEN_EPS = 1e-6

_NT = (((1,), (1,)), ((), ()))


def _nt(a, b):
    return lax.dot_general(a, b, _NT, preferred_element_type=jnp.float32)


def _nn(a, b):
    return jnp.dot(a, b, preferred_element_type=jnp.float32)


def _layernorm_bf16(x):
    m = jnp.mean(x, axis=-1, keepdims=True)
    xc = x - m
    v = jnp.mean(xc * xc, axis=-1, keepdims=True)
    return (xc * lax.rsqrt(v + LN_EPS)).astype(jnp.bfloat16)


def _fold_halves(x, op):
    return op(x, pltpu.roll(x, 4, 0))


def _feature_unit(p):
    p3 = p.reshape(NT10, 8, 128)
    mx = _fold_halves(jnp.max(p3, axis=0), jnp.maximum)
    mn = _fold_halves(jnp.min(p3, axis=0), jnp.minimum)
    ep = jnp.exp2(p3 - mx[None])
    en = jnp.exp2(mn[None] - p3)
    rp = 1.0 / _fold_halves(jnp.sum(ep, axis=0), jnp.add)
    rn = 1.0 / _fold_halves(jnp.sum(en, axis=0), jnp.add)
    phi = jnp.concatenate([ep * rp[None], en * rn[None]], axis=0)
    return phi.reshape(GF, 128)


def _kernel(x_hbm, wqkv_hbm, wphi_ref, wo_hbm, w1t_hbm, w2_hbm, o_ref,
            wqkv_ref, wo_ref, w1t_ref, w2_ref, sems, xbuf_ref, xsems,
            wt_ref, wflat_ref, phiq_ref, xs_ref, qkvt_ref, phik_ref, vt_ref, phin_ref,
            kvt_acc_ref, z_acc_ref, kvt_ref, zb_ref):
    t_id = pl.program_id(0)

    def wcopy(k):
        if k < 3:
            src = wqkv_hbm.at[:, pl.ds(k * D, D)]
            dst = wqkv_ref.at[:, pl.ds(k * D, D)]
        else:
            src, dst = ((wo_hbm, wo_ref), (w1t_hbm, w1t_ref),
                        (w2_hbm, w2_ref))[k - 3]
        return pltpu.make_async_copy(src, dst, sems.at[k])

    def xcopy(b):
        return pltpu.make_async_copy(
            x_hbm.at[pl.ds(b * TB, TB), :], xbuf_ref.at[b % 2], xsems.at[b % 2])

    def prep():
        wflat_ref[...] = jnp.zeros_like(wflat_ref)
        for e in range(DH):
            wflat_ref[pl.ds(e, H, stride=DH), pl.ds(0, DH)] = (
                wphi_ref[e].astype(jnp.float32).T)
        wflat = wflat_ref[...].astype(jnp.bfloat16)
        crow = lax.broadcasted_iota(jnp.int32, (2 * GV, 128), 0)
        dcol = lax.broadcasted_iota(jnp.int32, (2 * GV, 128), 1)
        rem = crow % GV
        dsel = (rem // 8) * 2 + (rem % 8) // 4
        sel = jnp.where(dsel == dcol, 1.0, 0.0).astype(jnp.bfloat16)
        crow = lax.broadcasted_iota(jnp.int32, (2 * GV, 256), 0)
        rcol = lax.broadcasted_iota(jnp.int32, (2 * GV, 256), 1)
        head_c = (crow // GV) * G4 + crow % G4
        pts = []
        for g in range(NG // 2):
            ptw = _nt(sel, wflat[g * 128:g * 128 + 256, :])
            head_r = (rcol + g * 128) // DH - g * 2 * G4
            pts.append(jnp.where(head_c == head_r, ptw, 0.0).astype(jnp.bfloat16))
        for part in range(2):
            wcopy(part).wait()
            for g in range(NG // 2):
                wt_ref[pl.ds(part * D + g * 2 * GV, 2 * GV), :] = (LOG2E * _nt(
                    pts[g], wqkv_ref[:, pl.ds(part * D + g * 128, 256)],
                )).astype(jnp.bfloat16)
        wcopy(2).wait()
        wt_ref[pl.ds(2 * D, D), :] = wqkv_ref[:, pl.ds(2 * D, D)].T

    def reset_acc():
        kvt_acc_ref[...] = jnp.zeros_like(kvt_acc_ref)
        z_acc_ref[...] = jnp.zeros_like(z_acc_ref)

    def finalize():
        crow = lax.broadcasted_iota(jnp.int32, (GV, GF), 0)
        fcol = lax.broadcasted_iota(jnp.int32, (GV, GF), 1)
        same_head = (crow // DH) == (fcol % G4)
        for g in range(NG):
            kvt_ref[g] = jnp.where(same_head, kvt_acc_ref[g], 0.0).astype(
                jnp.bfloat16)
        z = jnp.sum(z_acc_ref[...], axis=1, keepdims=True)
        zb_ref[...] = jnp.broadcast_to(z, zb_ref.shape)

    def front_den(blk):
        for g in range(NG):
            zt = zb_ref[pl.ds(g * GF, GF), :].reshape(2 * NT10, 8, 128)
            for j in range(NL):
                pq = phiq_ref[blk, pl.ds(g * GF, GF), pl.ds(j * 128, 128)]
                pq = pq.astype(jnp.float32).reshape(2 * NT10, 8, 128)
                den = _fold_halves(jnp.sum(pq * zt, axis=0), jnp.add) + DEN_EPS
                pn = (pq * (1.0 / den)[None]).reshape(GF, 128)
                phin_ref[pl.ds(g * GF, GF), pl.ds(j * 128, 128)] = (
                    pn.astype(jnp.bfloat16))

    def stage_a(blk):
        ot = jnp.concatenate(
            [_nn(kvt_ref[g], phin_ref[pl.ds(g * GF, GF), :])
             for g in range(NG)], axis=0)
        o = ot.astype(jnp.bfloat16).T
        x1 = xs_ref[blk] + _nn(o, wo_ref[...])
        xn1 = _layernorm_bf16(x1)
        hpre = _nt(xn1, w1t_ref[...])
        hact = (hpre * jax.nn.sigmoid(hpre)).astype(jnp.bfloat16)
        front_den((blk + 1) % NB)
        x2 = x1 + _nn(hact, w2_ref[...])
        xs_ref[blk] = x2

    def stage_bmm(blk):
        xn = _layernorm_bf16(xs_ref[blk])
        qkvt_ref[...] = _nt(wt_ref[...], xn)

    def feat_q(blk):
        for g in range(NG):
            for j in range(NL):
                phi = _feature_unit(
                    qkvt_ref[pl.ds(g * GV, GV), pl.ds(j * 128, 128)])
                phiq_ref[blk, pl.ds(g * GF, GF), pl.ds(j * 128, 128)] = (
                    phi.astype(jnp.bfloat16))

    def feat_kv():
        for g in range(NG):
            zsum = None
            for j in range(NL):
                phi = _feature_unit(
                    qkvt_ref[pl.ds(D + g * GV, GV), pl.ds(j * 128, 128)])
                phik_ref[pl.ds(g * GF, GF), pl.ds(j * 128, 128)] = (
                    phi.astype(jnp.bfloat16))
                zsum = phi if zsum is None else zsum + phi
            z_acc_ref[pl.ds(g * GF, GF), :] += zsum
        vt_ref[...] = qkvt_ref[pl.ds(2 * D, D), :].astype(jnp.bfloat16)

    def stage_bfeat(blk):
        feat_q(blk)
        feat_kv()

    def stage_bkv():
        for g in range(NG):
            kvt_acc_ref[g] += _nt(vt_ref[pl.ds(g * GV, GV), :],
                                  phik_ref[pl.ds(g * GF, GF), :])

    def zero_kv_operands():
        phik_ref[...] = jnp.zeros_like(phik_ref)
        vt_ref[...] = jnp.zeros_like(vt_ref)

    blk = t_id % NB

    @pl.when(t_id == 0)
    def _():
        for k in range(3):
            wcopy(k).start()
        xcopy(0).start()
        reset_acc()
        zero_kv_operands()
        prep()
        for k in range(3, 6):
            wcopy(k).start()

    @pl.when(t_id < NB)
    def _():
        xcopy(blk).wait()
        xs_ref[blk] = xbuf_ref[blk % 2].astype(jnp.float32)

    @pl.when(t_id + 1 < NB)
    def _():
        xcopy(blk + 1).start()

    @pl.when(jnp.logical_or(t_id == NB, t_id == 2 * NB))
    def _():
        stage_bkv()
        feat_kv()
        stage_bkv()
        feat_q(NB - 1)
        finalize()
        front_den(0)
        reset_acc()
        zero_kv_operands()

    @pl.when(t_id == NB)
    def _():
        for k in range(3, 6):
            wcopy(k).wait()

    @pl.when(t_id >= NB)
    def _():
        stage_a(blk)

    @pl.when(t_id >= 2 * NB)
    def _():
        o_ref[...] = xs_ref[blk].astype(o_ref.dtype)

    @pl.when(jnp.logical_and(blk == 0, t_id < 2 * NB))
    def _():
        stage_bmm(blk)

    @pl.when(jnp.logical_and(blk > 0, t_id < 2 * NB))
    def _():
        stage_bkv()
        stage_bfeat(blk - 1)
        stage_bmm(blk)


@jax.jit
def pallas_interleave_layers__linear_kernel_hedgehog__dense_activation_silu__prompt_kernel(
    A_x: jax.Array,
    A_wqkv: jax.Array,
    A_w_phi: jax.Array,
    A_wo: jax.Array,
    B_x: jax.Array,
    B_w1: jax.Array,
    B_w2: jax.Array,
):
    del B_x
    x2d = A_x.reshape(S, D)
    w1t = B_w1.T
    wphi_t = A_w_phi.transpose(1, 2, 0)

    hbm = pl.BlockSpec(memory_space=pl.ANY)
    grid_spec = pltpu.PrefetchScalarGridSpec(
        num_scalar_prefetch=0,
        grid=(NSTEP,),
        in_specs=[
            hbm,
            hbm,
            pl.BlockSpec((DH, DH, H), lambda t: (0, 0, 0)),
            hbm, hbm, hbm,
        ],
        out_specs=pl.BlockSpec((TB, D), lambda t: (jnp.maximum(t - 2 * NB, 0), 0)),
        scratch_shapes=[
            pltpu.VMEM((D, 3 * D), jnp.bfloat16),
            pltpu.VMEM((D, D), jnp.bfloat16),
            pltpu.VMEM((F, D), jnp.bfloat16),
            pltpu.VMEM((F, D), jnp.bfloat16),
            pltpu.SemaphoreType.DMA((6,)),
            pltpu.VMEM((2, TB, D), jnp.bfloat16),
            pltpu.SemaphoreType.DMA((2,)),
            pltpu.VMEM((3 * D, D), jnp.bfloat16),
            pltpu.VMEM((D, 128), jnp.float32),
            pltpu.VMEM((NB, 2 * D, TB), jnp.bfloat16),
            pltpu.VMEM((NB, TB, D), jnp.float32),
            pltpu.VMEM((3 * D, TB), jnp.float32),
            pltpu.VMEM((2 * D, TB), jnp.bfloat16),
            pltpu.VMEM((D, TB), jnp.bfloat16),
            pltpu.VMEM((2 * D, TB), jnp.bfloat16),
            pltpu.VMEM((NG, GV, GF), jnp.float32),
            pltpu.VMEM((2 * D, 128), jnp.float32),
            pltpu.VMEM((NG, GV, GF), jnp.bfloat16),
            pltpu.VMEM((2 * D, 128), jnp.float32),
        ],
    )
    out = pl.pallas_call(
        _kernel,
        grid_spec=grid_spec,
        out_shape=jax.ShapeDtypeStruct((S, D), jnp.bfloat16),
        compiler_params=pltpu.CompilerParams(
            dimension_semantics=("arbitrary",),
            vmem_limit_bytes=100 * 1024 * 1024,
        ),
    )(x2d, A_wqkv, wphi_t, A_wo, w1t, B_w2)
    return out.reshape(1, S, D)
```
